```python
import os as _os
_os.environ.setdefault("JAX_PLATFORMS", "cpu")
import jax
import jax.numpy as jnp

def _softmax(x, axis=-1):
    return jax.nn.softmax(x, axis=axis)
def _gelu(x):
    return jax.nn.gelu(x, approximate=True)
def _silu(x):
    return jax.nn.silu(x)
def _sigmoid(x):
    return jax.nn.sigmoid(x)
def _layernorm(x, axis=-1, eps=1e-5):
    m = jnp.mean(x, axis=axis, keepdims=True)
    v = jnp.var(x, axis=axis, keepdims=True)
    return (x - m) / jnp.sqrt(v + eps)
def _scatter_add(tgt, idx, src, axis=0):
    return tgt.at[idx].add(src)
def _segment_sum(src, seg, n):
    return jax.ops.segment_sum(src, seg, n)
class _Rng:
    def __init__(self, key):
        self._k = key
    def _next(self):
        self._k, sub = jax.random.split(self._k)
        return sub
    def normal(self, shape):
        return jax.random.normal(self._next(), shape, dtype=jnp.bfloat16)
    def randint(self, lo, hi, shape):
        return jax.random.randint(self._next(), shape, lo, hi, dtype=jnp.int32)
    def uniform(self, shape, lo=0.0, hi=1.0):
        return jax.random.uniform(self._next(), shape, jnp.bfloat16, lo, hi)
    def permutation(self, n):
        return jax.random.permutation(self._next(), n)


kernel_name = 'interleave_layers__spectral_gfnet__dense_activation_gelu__prompt'

def setup_inputs():
    _rng = _Rng(jax.random.key(int.from_bytes(__import__("os").urandom(4), "little")))
    _w = (lambda a: (lambda t: t.astype(jnp.bfloat16) if jnp.issubdtype(t.dtype, jnp.floating) else t)(jnp.asarray(a)))
    def _A_setup():
        B, S, D = 1, 2048, 640
        Df = D // 2 + 1
        return {
            "x": _w((lambda *s: _rng.normal(s) * 0.05)(B, S, D)),
            "w_r": _w((lambda *s: _rng.normal(s) * 0.2)(S, Df) * 0.02),
            "w_i": _w((lambda *s: _rng.normal(s) * 0.2)(S, Df) * 0.02),
        }
    _A_in = _A_setup()

    def _B_setup():
        B, S, D, F = 1, 2048, 640, 1728
        return {
            "x": _w((lambda *s: _rng.normal(s) * 0.05)(B, S, D)),
            "w1": _w((lambda *s: _rng.normal(s) * 0.1)(D, F) * (D ** -0.5)),
            "b1": _w((lambda *s: _rng.normal(s) * 0.1)(F) * 0.01),
            "w2": _w((lambda *s: _rng.normal(s) * 0.1)(F, D) * (F ** -0.5)),
            "b2": _w((lambda *s: _rng.normal(s) * 0.1)(D) * 0.01),
        }
    _B_in = _B_setup()

    return {
        "A_x": _A_in["x"],
        "A_w_r": _A_in["w_r"],
        "A_w_i": _A_in["w_i"],
        "B_x": _B_in["x"],
        "B_w1": _B_in["w1"],
        "B_b1": _B_in["b1"],
        "B_w2": _B_in["w2"],
        "B_b2": _B_in["b2"],
    }

def reference(A_x, A_w_r, A_w_i, B_x, B_w1, B_b1, B_w2, B_b2):
    def _A_ref(x, w_r, w_i):
        B, S, D = x.shape
        X = (lambda x, axes=(-2,-1): jnp.fft.rfft2(x.astype(jnp.float32), axes=axes))(x, axes=(-2, -1))
        W = w_r + 1j * w_i
        X = X * W
        y = (lambda x, s, axes=(-2,-1): jnp.fft.irfft2(x, s=s, axes=axes).astype(jnp.bfloat16))(X, (S, D), axes=(-2, -1))
        return y

    def _B_ref(x, w1, b1, w2, b2):
        h = jnp.einsum("bsd,df->bsf", x, w1) + b1
        h = _gelu(h)
        return jnp.einsum("bsf,fd->bsd", h, w2) + b2

    x = A_x
    x = x + _A_ref(_layernorm(x, axis=-1), A_w_r, A_w_i)
    x = x + _B_ref(_layernorm(x, axis=-1), B_w1, B_b1, B_w2, B_b2)
    x = x + _A_ref(_layernorm(x, axis=-1), A_w_r, A_w_i)
    x = x + _B_ref(_layernorm(x, axis=-1), B_w1, B_b1, B_w2, B_b2)
    return x
```

```python
import functools
import math

import jax
import jax.numpy as jnp
import numpy as np
import jax.experimental.pallas as pl
import jax.experimental.pallas.tpu as pltpu

S, D, F = 2048, 640, 1728
DF = D // 2 + 1
L = 128
DP = 3 * L
N1, N2 = 16, 128
ROWS = 512
EPS = 1e-5

C72, S72 = math.cos(2 * math.pi / 5), math.sin(2 * math.pi / 5)
C144, S144 = math.cos(4 * math.pi / 5), math.sin(4 * math.pi / 5)


@functools.lru_cache(maxsize=None)
def _dft_constants():
    n2 = np.arange(L)[:, None]

    def theta(k):
        return 2.0 * np.pi * ((n2 * k[None, :]) % D) / D

    k0 = 5 * np.arange(65)
    t0 = theta(k0)
    m0 = np.zeros((L, 2 * L))
    m0[:, :65] = np.cos(t0)
    m0[:, L:L + 65] = -np.sin(t0)

    def fwd_pair(ka, kb):
        ta, tb = theta(ka), theta(kb)
        m = np.zeros((2 * L, 2 * L))
        m[:L, 0:64], m[L:, 0:64] = np.cos(ta), np.sin(ta)
        m[:L, 64:128], m[L:, 64:128] = np.cos(tb), -np.sin(tb)
        m[:L, 128:192], m[L:, 128:192] = -np.sin(ta), np.cos(ta)
        m[:L, 192:256], m[L:, 192:256] = -np.sin(tb), -np.cos(tb)
        return m

    kk = np.arange(64)
    m14 = fwd_pair(1 + 5 * kk, 4 + 5 * kk)
    m23 = fwd_pair(2 + 5 * kk, 3 + 5 * kk)
    fwd = np.concatenate([np.concatenate([m0, np.zeros((L, 2 * L))], 0)[None],
                          m14[None], m23[None]], 0)

    scale = 1.0 / (S * D)
    c = np.full((65,), 2.0)
    c[0] = c[-1] = 1.0
    i0 = np.zeros((2 * L, 2 * L))
    i0[:65, :L] = (c[:, None] * np.cos(t0.T))
    i0[L:L + 65, :L] = (-c[:, None] * np.sin(t0.T))

    def inv_pair(ka, kb):
        ta, tb = theta(ka).T, theta(kb).T
        m = np.zeros((2 * L, 2 * L))
        m[0:64, :L], m[0:64, L:] = np.cos(ta), np.sin(ta)
        m[64:128, :L], m[64:128, L:] = np.cos(tb), -np.sin(tb)
        m[128:192, :L], m[128:192, L:] = -np.sin(ta), np.cos(ta)
        m[192:256, :L], m[192:256, L:] = -np.sin(tb), -np.cos(tb)
        return 2.0 * m

    inv = np.stack([i0, inv_pair(1 + 5 * kk, 4 + 5 * kk),
                    inv_pair(2 + 5 * kk, 3 + 5 * kk)], 0) * scale
    a = np.arange(N1)
    f16 = np.exp(-2j * np.pi * np.outer(a, a) / N1)
    kf = np.kron(f16, np.eye(8))
    rad = np.stack([np.concatenate([kf.real, kf.imag], axis=0),
                    np.concatenate([kf.real, -kf.imag], axis=0)], 0)
    k1 = np.arange(N1)[:, None, None]
    k2 = np.arange(N2)[None, :, None]
    nn = np.arange(N2)[None, None, :]
    angs = 2.0 * np.pi * ((nn * (k1 + N1 * k2)) % S) / S
    g_f = np.concatenate([np.cos(angs), -np.sin(angs)], axis=1)
    angs_t = np.transpose(angs, (0, 2, 1))
    g_i = np.concatenate([np.cos(angs_t), np.sin(angs_t)], axis=1)
    return tuple(x.astype(np.float32).astype(jnp.bfloat16)
                 for x in (fwd, inv, g_f, g_i))


def _ln(x):
    m = jnp.mean(x, axis=-1, keepdims=True)
    xc = x - m
    v = jnp.mean(xc * xc, axis=-1, keepdims=True)
    return xc * jax.lax.rsqrt(v + EPS)


def _fft_list(v, sign):
    n = len(v)
    if n == 1:
        return v
    ev = _fft_list(v[0::2], sign)
    od = _fft_list(v[1::2], sign)
    out = [None] * n
    for k in range(n // 2):
        orr, oi = od[k]
        if k == 0:
            tr, ti = orr, oi
        elif 4 * k == n:
            tr, ti = (-oi, orr) if sign > 0 else (oi, -orr)
        else:
            wr = math.cos(2 * math.pi * k / n)
            wi = sign * math.sin(2 * math.pi * k / n)
            tr = orr * wr - oi * wi
            ti = orr * wi + oi * wr
        er, ei = ev[k]
        out[k] = (er + tr, ei + ti)
        out[k + n // 2] = (er - tr, ei - ti)
    return out


def _cmul_split(p):
    re = p[:N2, :DP] - p[N2:, DP:]
    im = p[:N2, DP:] + p[N2:, :DP]
    return re, im


def _kernel(x_hbm, wr_hbm, wi_hbm, w1t_hbm, b1_ref, w2_hbm, b2_ref,
            fwd_hbm, inv_hbm, gf_hbm, gi_hbm,
            o_hbm,
            xin_ref, wr_ref, wi_ref, w1t_ref, w2_ref,
            fwd_ref, inv_ref, gf_ref, gi_ref,
            xs_ref, z_ref, wn_ref, tmp_ref, sems, osems):
    f32 = jnp.float32
    bf16 = jnp.bfloat16
    nt = S // ROWS

    pairs = [(x_hbm, xin_ref), (fwd_hbm, fwd_ref), (gf_hbm, gf_ref),
             (wr_hbm, wr_ref), (wi_hbm, wi_ref), (gi_hbm, gi_ref), (inv_hbm, inv_ref),
             (w1t_hbm, w1t_ref), (w2_hbm, w2_ref)]
    copies = [pltpu.make_async_copy(s, d, sems.at[i]) for i, (s, d) in enumerate(pairs)]
    (c_x, c_fwd, c_gf, c_wr, c_wi, c_gi, c_inv, c_w1, c_w2) = copies
    c_x.start()
    c_fwd.start()

    def out_copy(t):
        r = pl.multiple_of(t * ROWS, ROWS)
        return pltpu.make_async_copy(xin_ref.at[pl.ds(r, ROWS), :],
                                     o_hbm.at[pl.ds(r, ROWS), :], osems.at[t])

    def dot(a, b):
        return jnp.dot(a, b, preferred_element_type=f32)

    def d_forward(x, r):
        xn = _ln(x)
        c0, c1, c2, c3, c4 = [xn[:, i * L:(i + 1) * L] for i in range(5)]
        s14, d14 = c1 + c4, c1 - c4
        s23, d23 = c2 + c3, c2 - c3
        a0 = c0 + s14 + s23
        a1 = jnp.concatenate([c0 + C72 * s14 + C144 * s23,
                              -(S72 * d14 + S144 * d23)], axis=1)
        a2 = jnp.concatenate([c0 + C144 * s14 + C72 * s23,
                              -(S144 * d14 - S72 * d23)], axis=1)
        p0 = dot(a0.astype(bf16), fwd_ref[0, :L, :])
        p1 = dot(a1.astype(bf16), fwd_ref[1])
        p2 = dot(a2.astype(bf16), fwd_ref[2])
        for g, p in enumerate((p0, p1, p2)):
            z_ref[pl.ds(r, ROWS), g * L:(g + 1) * L] = p[:, :L]
            z_ref[pl.ds(r, ROWS), DP + g * L:DP + (g + 1) * L] = p[:, L:]

    def d_inverse(r):
        q = []
        for g in range(3):
            yy = jnp.concatenate(
                [z_ref[pl.ds(r, ROWS), g * L:(g + 1) * L],
                 z_ref[pl.ds(r, ROWS), DP + g * L:DP + (g + 1) * L]], axis=1).astype(bf16)
            if g == 0:
                q.append(dot(yy, inv_ref[0, :, :L]))
            else:
                q.append(dot(yy, inv_ref[g]))
        b0 = q[0]
        p1, q1 = q[1][:, :L], q[1][:, L:]
        p2, q2 = q[2][:, :L], q[2][:, L:]
        ys = [b0 + p1 + p2,
              b0 + C72 * p1 - S72 * q1 + C144 * p2 - S144 * q2,
              b0 + C144 * p1 - S144 * q1 + C72 * p2 + S72 * q2,
              b0 + C144 * p1 + S144 * q1 + C72 * p2 - S72 * q2,
              b0 + C72 * p1 + S72 * q1 + C144 * p2 + S144 * q2]
        return jnp.concatenate(ys, axis=1)

    def radix_step(sign):
        def body(j, c):
            r = pl.multiple_of(j * 8, 8)
            v = [(z_ref[pl.ds(N2 * n1 + r, 8), :DP], z_ref[pl.ds(N2 * n1 + r, 8), DP:])
                 for n1 in range(N1)]
            v = _fft_list(v, sign)
            for n1 in range(N1):
                z_ref[pl.ds(N2 * n1 + r, 8), :DP] = v[n1][0]
                z_ref[pl.ds(N2 * n1 + r, 8), DP:] = v[n1][1]
            return c
        jax.lax.fori_loop(0, N2 // 8, body, 0)

    def t_body(b, c):
        r = pl.multiple_of(b * N2, N2)
        for h, src in enumerate((wr_ref, wi_ref)):
            tmp_ref[pl.ds(0, DF), :] = src[:, pl.ds(r, N2)].astype(f32)
            cls = [tmp_ref[pl.ds(k, 64, stride=5), :] for k in range(5)]
            g0 = jnp.concatenate(
                [cls[0], tmp_ref[pl.ds(320, 1), :], jnp.zeros((63, L), f32)], axis=0)
            g1 = jnp.concatenate([cls[1], cls[4]], axis=0)
            g2 = jnp.concatenate([cls[2], cls[3]], axis=0)
            for g, blk in enumerate((g0, g1, g2)):
                wn_ref[3 * h + g, pl.ds(r, N2), :] = blk.T
        return c

    def c_body(k1, c):
        r = pl.multiple_of(k1 * N2, N2)
        slab = z_ref[pl.ds(r, N2), :].astype(bf16)
        re, im = _cmul_split(dot(gf_ref[k1], slab))
        wr = jnp.concatenate(
            [wn_ref[g, pl.ds(k1, N2, stride=N1), :] for g in range(3)], axis=1)
        wi = jnp.concatenate(
            [wn_ref[3 + g, pl.ds(k1, N2, stride=N1), :] for g in range(3)], axis=1)
        yr = re * wr - im * wi
        yi = re * wi + im * wr
        y = jnp.concatenate([yr, yi], axis=1).astype(bf16)
        re, im = _cmul_split(dot(gi_ref[k1], y))
        z_ref[pl.ds(r, N2), :DP] = re
        z_ref[pl.ds(r, N2), DP:] = im
        return c

    def spectral_s(first):
        radix_step(-1)
        if first:
            c_wr.wait(); c_wi.wait()
            jax.lax.fori_loop(0, S // N2, t_body, 0)
            c_gf.wait(); c_gi.wait()
        jax.lax.fori_loop(0, N1, c_body, 0)
        radix_step(+1)

    def first_body(t, c):
        r = pl.multiple_of(t * ROWS, ROWS)
        x = xin_ref[pl.ds(r, ROWS), :].astype(f32)
        xs_ref[pl.ds(r, ROWS), :] = x
        d_forward(x, r)
        return c

    def row_phase(last):
        def body(t, c):
            r = pl.multiple_of(t * ROWS, ROWS)
            x = xs_ref[pl.ds(r, ROWS), :] + d_inverse(r)
            xn = _ln(x).astype(bf16)
            h = jax.lax.dot_general(xn, w1t_ref[...], (((1,), (1,)), ((), ())),
                                    preferred_element_type=f32)
            h = h + b1_ref[...].astype(f32)
            h = jax.nn.gelu(h, approximate=True).astype(bf16)
            x = x + (dot(h, w2_ref[...]) + b2_ref[...].astype(f32))
            if last:
                xin_ref[pl.ds(r, ROWS), :] = x.astype(bf16)
                out_copy(t).start()
            else:
                xs_ref[pl.ds(r, ROWS), :] = x
                d_forward(x, r)
            return c
        jax.lax.fori_loop(0, nt, body, 0)

    c_x.wait()
    c_fwd.wait()
    for cp in copies[2:]:
        cp.start()
    jax.lax.fori_loop(0, nt, first_body, 0)
    spectral_s(True)
    c_inv.wait(); c_w1.wait(); c_w2.wait()
    row_phase(False)
    spectral_s(False)
    row_phase(True)
    for t in range(nt):
        out_copy(t).wait()


@jax.jit
def pallas_interleave_layers__spectral_gfnet__dense_activation_gelu__prompt_kernel(
    A_x: jax.Array,
    A_w_r: jax.Array,
    A_w_i: jax.Array,
    B_x: jax.Array,
    B_w1: jax.Array,
    B_b1: jax.Array,
    B_w2: jax.Array,
    B_b2: jax.Array,
):
    del B_x
    x = A_x.reshape(S, D)

    wr = A_w_r.T
    wi = A_w_i.T
    consts = _dft_constants()
    bf16 = jnp.bfloat16
    any_spec = pl.BlockSpec(memory_space=pl.ANY)
    vmem_spec = pl.BlockSpec(memory_space=pltpu.VMEM)
    out = pl.pallas_call(
        _kernel,
        out_shape=jax.ShapeDtypeStruct((S, D), A_x.dtype),
        in_specs=[any_spec, any_spec, any_spec, any_spec, vmem_spec, any_spec, vmem_spec]
        + [any_spec] * 4,
        out_specs=any_spec,
        scratch_shapes=[
            pltpu.VMEM((S, D), bf16),
            pltpu.VMEM((DF, S), bf16),
            pltpu.VMEM((DF, S), bf16),
            pltpu.VMEM((F, D), bf16),
            pltpu.VMEM((F, D), bf16),
        ] + [pltpu.VMEM(c.shape, bf16) for c in consts] + [
            pltpu.VMEM((S, D), jnp.float32),
            pltpu.VMEM((S, 2 * DP), jnp.float32),
            pltpu.VMEM((6, S, L), jnp.float32),
            pltpu.VMEM((328, L), jnp.float32),
            pltpu.SemaphoreType.DMA((9,)),
            pltpu.SemaphoreType.DMA((S // ROWS,)),
        ],
        compiler_params=pltpu.CompilerParams(vmem_limit_bytes=100 * 1024 * 1024),
    )(x, wr, wi, B_w1.T, B_b1.reshape(1, F), B_w2, B_b2.reshape(1, D), *consts)
    return out.reshape(1, S, D)
```

```python
import functools
import math

import jax
import jax.numpy as jnp
import numpy as np
import jax.experimental.pallas as pl
import jax.experimental.pallas.tpu as pltpu

S, D, F = 2048, 640, 1728
DF = D // 2 + 1
L = 128
DP = 3 * L
N1, N2 = 16, 128
ROWS = 512
EPS = 1e-5

C72, S72 = math.cos(2 * math.pi / 5), math.sin(2 * math.pi / 5)
C144, S144 = math.cos(4 * math.pi / 5), math.sin(4 * math.pi / 5)


@functools.lru_cache(maxsize=None)
def _dft_constants():
    n2 = np.arange(L)[:, None]

    def theta(k):
        return 2.0 * np.pi * ((n2 * k[None, :]) % D) / D

    k0 = 5 * np.arange(65)
    t0 = theta(k0)
    m0 = np.zeros((L, 2 * L))
    m0[:, :65] = np.cos(t0)
    m0[:, L:L + 65] = -np.sin(t0)

    def fwd_pair(ka, kb):
        ta, tb = theta(ka), theta(kb)
        m = np.zeros((2 * L, 2 * L))
        m[:L, 0:64], m[L:, 0:64] = np.cos(ta), np.sin(ta)
        m[:L, 64:128], m[L:, 64:128] = np.cos(tb), -np.sin(tb)
        m[:L, 128:192], m[L:, 128:192] = -np.sin(ta), np.cos(ta)
        m[:L, 192:256], m[L:, 192:256] = -np.sin(tb), -np.cos(tb)
        return m

    kk = np.arange(64)
    m14 = fwd_pair(1 + 5 * kk, 4 + 5 * kk)
    m23 = fwd_pair(2 + 5 * kk, 3 + 5 * kk)
    fwd = np.concatenate([np.concatenate([m0, np.zeros((L, 2 * L))], 0)[None],
                          m14[None], m23[None]], 0)

    scale = 1.0 / (S * D)
    c = np.full((65,), 2.0)
    c[0] = c[-1] = 1.0
    i0 = np.zeros((2 * L, 2 * L))
    i0[:65, :L] = (c[:, None] * np.cos(t0.T))
    i0[L:L + 65, :L] = (-c[:, None] * np.sin(t0.T))

    def inv_pair(ka, kb):
        ta, tb = theta(ka).T, theta(kb).T
        m = np.zeros((2 * L, 2 * L))
        m[0:64, :L], m[0:64, L:] = np.cos(ta), np.sin(ta)
        m[64:128, :L], m[64:128, L:] = np.cos(tb), -np.sin(tb)
        m[128:192, :L], m[128:192, L:] = -np.sin(ta), np.cos(ta)
        m[192:256, :L], m[192:256, L:] = -np.sin(tb), -np.cos(tb)
        return 2.0 * m

    inv = np.stack([i0, inv_pair(1 + 5 * kk, 4 + 5 * kk),
                    inv_pair(2 + 5 * kk, 3 + 5 * kk)], 0) * scale
    a = np.arange(N1)
    f16 = np.exp(-2j * np.pi * np.outer(a, a) / N1)
    kf = np.kron(f16, np.eye(8))
    rad = np.stack([np.concatenate([kf.real, kf.imag], axis=0),
                    np.concatenate([kf.real, -kf.imag], axis=0)], 0)
    k1 = np.arange(N1)[:, None, None]
    k2 = np.arange(N2)[None, :, None]
    nn = np.arange(N2)[None, None, :]
    angs = 2.0 * np.pi * ((nn * (k1 + N1 * k2)) % S) / S
    g_f = np.concatenate([np.cos(angs), -np.sin(angs)], axis=1)
    angs_t = np.transpose(angs, (0, 2, 1))
    g_i = np.concatenate([np.cos(angs_t), np.sin(angs_t)], axis=1)
    return tuple(x.astype(np.float32).astype(jnp.bfloat16)
                 for x in (fwd, inv, g_f, g_i))


def _ln(x):
    m = jnp.mean(x, axis=-1, keepdims=True)
    xc = x - m
    v = jnp.mean(xc * xc, axis=-1, keepdims=True)
    return xc * jax.lax.rsqrt(v + EPS)


def _fft_list(v, sign):
    n = len(v)
    if n == 1:
        return v
    ev = _fft_list(v[0::2], sign)
    od = _fft_list(v[1::2], sign)
    out = [None] * n
    for k in range(n // 2):
        orr, oi = od[k]
        if k == 0:
            tr, ti = orr, oi
        elif 4 * k == n:
            tr, ti = (-oi, orr) if sign > 0 else (oi, -orr)
        else:
            wr = math.cos(2 * math.pi * k / n)
            wi = sign * math.sin(2 * math.pi * k / n)
            tr = orr * wr - oi * wi
            ti = orr * wi + oi * wr
        er, ei = ev[k]
        out[k] = (er + tr, ei + ti)
        out[k + n // 2] = (er - tr, ei - ti)
    return out


def _cmul_split(p):
    re = p[:N2, :DP] - p[N2:, DP:]
    im = p[:N2, DP:] + p[N2:, :DP]
    return re, im


def _kernel(x_hbm, wr_hbm, wi_hbm, w1t_hbm, b1_ref, w2_hbm, b2_ref,
            fwd_hbm, inv_hbm, gf_hbm, gi_hbm,
            o_hbm,
            xin_ref, wr_ref, wi_ref, w1t_ref, w2_ref,
            fwd_ref, inv_ref, gf_ref, gi_ref,
            xs_ref, z_ref, wn_ref, tmp_ref, sems, osems):
    f32 = jnp.float32
    bf16 = jnp.bfloat16
    nt = S // ROWS

    pairs = [(x_hbm, xin_ref), (fwd_hbm, fwd_ref), (gf_hbm, gf_ref),
             (wr_hbm, wr_ref), (wi_hbm, wi_ref), (gi_hbm, gi_ref), (inv_hbm, inv_ref),
             (w1t_hbm, w1t_ref), (w2_hbm, w2_ref)]
    copies = [pltpu.make_async_copy(s, d, sems.at[i]) for i, (s, d) in enumerate(pairs)]
    (c_x, c_fwd, c_gf, c_wr, c_wi, c_gi, c_inv, c_w1, c_w2) = copies
    c_x.start()
    c_fwd.start()

    def out_copy(t):
        r = pl.multiple_of(t * ROWS, ROWS)
        return pltpu.make_async_copy(xin_ref.at[pl.ds(r, ROWS), :],
                                     o_hbm.at[pl.ds(r, ROWS), :], osems.at[t])

    def dot(a, b):
        return jnp.dot(a, b, preferred_element_type=f32)

    def d_forward(x, r):
        xn = _ln(x)
        c0, c1, c2, c3, c4 = [xn[:, i * L:(i + 1) * L] for i in range(5)]
        s14, d14 = c1 + c4, c1 - c4
        s23, d23 = c2 + c3, c2 - c3
        a0 = c0 + s14 + s23
        a1 = jnp.concatenate([c0 + C72 * s14 + C144 * s23,
                              -(S72 * d14 + S144 * d23)], axis=1)
        a2 = jnp.concatenate([c0 + C144 * s14 + C72 * s23,
                              -(S144 * d14 - S72 * d23)], axis=1)
        p0 = dot(a0.astype(bf16), fwd_ref[0, :L, :])
        p1 = dot(a1.astype(bf16), fwd_ref[1])
        p2 = dot(a2.astype(bf16), fwd_ref[2])
        for g, p in enumerate((p0, p1, p2)):
            z_ref[pl.ds(r, ROWS), g * L:(g + 1) * L] = p[:, :L]
            z_ref[pl.ds(r, ROWS), DP + g * L:DP + (g + 1) * L] = p[:, L:]

    def d_inverse(r):
        q = []
        for g in range(3):
            yy = jnp.concatenate(
                [z_ref[pl.ds(r, ROWS), g * L:(g + 1) * L],
                 z_ref[pl.ds(r, ROWS), DP + g * L:DP + (g + 1) * L]], axis=1).astype(bf16)
            if g == 0:
                q.append(dot(yy, inv_ref[0, :, :L]))
            else:
                q.append(dot(yy, inv_ref[g]))
        b0 = q[0]
        p1, q1 = q[1][:, :L], q[1][:, L:]
        p2, q2 = q[2][:, :L], q[2][:, L:]
        ys = [b0 + p1 + p2,
              b0 + C72 * p1 - S72 * q1 + C144 * p2 - S144 * q2,
              b0 + C144 * p1 - S144 * q1 + C72 * p2 + S72 * q2,
              b0 + C144 * p1 + S144 * q1 + C72 * p2 - S72 * q2,
              b0 + C72 * p1 + S72 * q1 + C144 * p2 + S144 * q2]
        return jnp.concatenate(ys, axis=1)

    def radix_step(sign, with_t=False):
        def body(j, c):
            r = pl.multiple_of(j * 8, 8)
            v = [(z_ref[pl.ds(N2 * n1 + r, 8), :DP], z_ref[pl.ds(N2 * n1 + r, 8), DP:])
                 for n1 in range(N1)]
            v = _fft_list(v, sign)
            for n1 in range(N1):
                z_ref[pl.ds(N2 * n1 + r, 8), :DP] = v[n1][0]
                z_ref[pl.ds(N2 * n1 + r, 8), DP:] = v[n1][1]
            if with_t:
                t_body(j, 0)
            return c
        jax.lax.fori_loop(0, N2 // 8, body, 0)

    def t_body(b, c):
        r = pl.multiple_of(b * N2, N2)
        for h, src in enumerate((wr_ref, wi_ref)):
            tmp_ref[pl.ds(0, DF), :] = src[:, pl.ds(r, N2)].astype(f32)
            cls = [tmp_ref[pl.ds(k, 64, stride=5), :] for k in range(5)]
            g0 = jnp.concatenate(
                [cls[0], tmp_ref[pl.ds(320, 1), :], jnp.zeros((63, L), f32)], axis=0)
            g1 = jnp.concatenate([cls[1], cls[4]], axis=0)
            g2 = jnp.concatenate([cls[2], cls[3]], axis=0)
            for g, blk in enumerate((g0, g1, g2)):
                wn_ref[3 * h + g, pl.ds(r, N2), :] = blk.T
        return c

    def c_body(k1, c):
        r = pl.multiple_of(k1 * N2, N2)
        slab = z_ref[pl.ds(r, N2), :].astype(bf16)
        re, im = _cmul_split(dot(gf_ref[k1], slab))
        wr = jnp.concatenate(
            [wn_ref[g, pl.ds(k1, N2, stride=N1), :] for g in range(3)], axis=1)
        wi = jnp.concatenate(
            [wn_ref[3 + g, pl.ds(k1, N2, stride=N1), :] for g in range(3)], axis=1)
        yr = re * wr - im * wi
        yi = re * wi + im * wr
        y = jnp.concatenate([yr, yi], axis=1).astype(bf16)
        re, im = _cmul_split(dot(gi_ref[k1], y))
        z_ref[pl.ds(r, N2), :DP] = re
        z_ref[pl.ds(r, N2), DP:] = im
        return c

    def spectral_s(first):
        if first:
            c_wr.wait(); c_wi.wait()
        radix_step(-1, with_t=first)
        if first:
            c_gf.wait(); c_gi.wait()
        jax.lax.fori_loop(0, N1, c_body, 0)
        radix_step(+1)

    def first_body(t, c):
        r = pl.multiple_of(t * ROWS, ROWS)
        x = xin_ref[pl.ds(r, ROWS), :].astype(f32)
        xs_ref[pl.ds(r, ROWS), :] = x
        d_forward(x, r)
        return c

    def row_phase(last):
        def body(t, c):
            r = pl.multiple_of(t * ROWS, ROWS)
            x = xs_ref[pl.ds(r, ROWS), :] + d_inverse(r)
            xn = _ln(x).astype(bf16)
            h = jax.lax.dot_general(xn, w1t_ref[...], (((1,), (1,)), ((), ())),
                                    preferred_element_type=f32)
            h = h + b1_ref[...].astype(f32)
            h = jax.nn.gelu(h, approximate=True).astype(bf16)
            x = x + (dot(h, w2_ref[...]) + b2_ref[...].astype(f32))
            if last:
                xin_ref[pl.ds(r, ROWS), :] = x.astype(bf16)
                out_copy(t).start()
            else:
                xs_ref[pl.ds(r, ROWS), :] = x
                d_forward(x, r)
            return c
        jax.lax.fori_loop(0, nt, body, 0)

    c_x.wait()
    c_fwd.wait()
    for cp in copies[2:]:
        cp.start()
    jax.lax.fori_loop(0, nt, first_body, 0)
    spectral_s(True)
    c_inv.wait(); c_w1.wait(); c_w2.wait()
    row_phase(False)
    spectral_s(False)
    row_phase(True)
    for t in range(nt):
        out_copy(t).wait()


@jax.jit
def pallas_interleave_layers__spectral_gfnet__dense_activation_gelu__prompt_kernel(
    A_x: jax.Array,
    A_w_r: jax.Array,
    A_w_i: jax.Array,
    B_x: jax.Array,
    B_w1: jax.Array,
    B_b1: jax.Array,
    B_w2: jax.Array,
    B_b2: jax.Array,
):
    del B_x
    x = A_x.reshape(S, D)

    wr = A_w_r.T
    wi = A_w_i.T
    consts = _dft_constants()
    bf16 = jnp.bfloat16
    any_spec = pl.BlockSpec(memory_space=pl.ANY)
    vmem_spec = pl.BlockSpec(memory_space=pltpu.VMEM)
    out = pl.pallas_call(
        _kernel,
        out_shape=jax.ShapeDtypeStruct((S, D), A_x.dtype),
        in_specs=[any_spec, any_spec, any_spec, any_spec, vmem_spec, any_spec, vmem_spec]
        + [any_spec] * 4,
        out_specs=any_spec,
        scratch_shapes=[
            pltpu.VMEM((S, D), bf16),
            pltpu.VMEM((DF, S), bf16),
            pltpu.VMEM((DF, S), bf16),
            pltpu.VMEM((F, D), bf16),
            pltpu.VMEM((F, D), bf16),
        ] + [pltpu.VMEM(c.shape, bf16) for c in consts] + [
            pltpu.VMEM((S, D), jnp.float32),
            pltpu.VMEM((S, 2 * DP), jnp.float32),
            pltpu.VMEM((6, S, L), jnp.float32),
            pltpu.VMEM((328, L), jnp.float32),
            pltpu.SemaphoreType.DMA((9,)),
            pltpu.SemaphoreType.DMA((S // ROWS,)),
        ],
        compiler_params=pltpu.CompilerParams(vmem_limit_bytes=100 * 1024 * 1024),
    )(x, wr, wi, B_w1.T, B_b1.reshape(1, F), B_w2, B_b2.reshape(1, D), *consts)
    return out.reshape(1, S, D)
```
